```python
import os as _os
_os.environ.setdefault("JAX_PLATFORMS", "cpu")
import jax
import jax.numpy as jnp

def _softmax(x, axis=-1):
    return jax.nn.softmax(x, axis=axis)
def _gelu(x):
    return jax.nn.gelu(x, approximate=True)
def _silu(x):
    return jax.nn.silu(x)
def _sigmoid(x):
    return jax.nn.sigmoid(x)
def _layernorm(x, axis=-1, eps=1e-5):
    m = jnp.mean(x, axis=axis, keepdims=True)
    v = jnp.var(x, axis=axis, keepdims=True)
    return (x - m) / jnp.sqrt(v + eps)
def _scatter_add(tgt, idx, src, axis=0):
    return tgt.at[idx].add(src)
def _segment_sum(src, seg, n):
    return jax.ops.segment_sum(src, seg, n)
class _Rng:
    def __init__(self, key):
        self._k = key
    def _next(self):
        self._k, sub = jax.random.split(self._k)
        return sub
    def normal(self, shape):
        return jax.random.normal(self._next(), shape, dtype=jnp.bfloat16)
    def randint(self, lo, hi, shape):
        return jax.random.randint(self._next(), shape, lo, hi, dtype=jnp.int32)
    def uniform(self, shape, lo=0.0, hi=1.0):
        return jax.random.uniform(self._next(), shape, jnp.bfloat16, lo, hi)
    def permutation(self, n):
        return jax.random.permutation(self._next(), n)


kernel_name = 'standalone__mha_softmax__near_ridge'

def setup_inputs():
    _rng = _Rng(jax.random.key(int.from_bytes(__import__("os").urandom(4), "little")))
    _w = (lambda a: (lambda t: t.astype(jnp.bfloat16) if jnp.issubdtype(t.dtype, jnp.floating) else t)(jnp.asarray(a)))
    B, H, Sq, Sk, D = 16, 16, 256, 256, 256
    return {
        "q": _w((lambda *s: _rng.normal(s) * 0.4)(B, H, Sq, D)),
        "k": _w((lambda *s: _rng.normal(s) * 0.4)(B, H, Sk, D)),
        "v": _w((lambda *s: _rng.normal(s) * 0.05)(B, H, Sk, D)),
    }

def reference(q, k, v):
    scale = q.shape[-1] ** -0.5
    scores = jnp.einsum("bhqd,bhkd->bhqk", q, k) * scale
    p = _softmax(scores, axis=-1)
    return jnp.einsum("bhqk,bhkd->bhqd", p, v)
```

```python
import jax
import jax.numpy as jnp
from jax import lax
import jax.experimental.pallas as pl
import jax.experimental.pallas.tpu as pltpu

_LOG2E = 1.4426950408889634

_CH = 2
_W = 4
_R = 8
_E = 2
_WCH = 8


def _head_attention(q, k, v, c):
    s = lax.dot_general(
        q, k, (((1,), (1,)), ((), ())), preferred_element_type=jnp.float32
    )
    m = jnp.max(s, axis=-1, keepdims=True)
    p = jnp.exp2((s - m) * c)
    l = jnp.sum(p, axis=-1, keepdims=True)
    o = jnp.dot(p.astype(v.dtype), v, preferred_element_type=jnp.float32)
    return (o * (1.0 / l)).astype(v.dtype)


@jax.jit
def pallas_standalone__mha_softmax__near_ridge_kernel(
    q: jax.Array,
    k: jax.Array,
    v: jax.Array,
):
    B, H, Sq, D = q.shape
    Sk = k.shape[2]
    N = B * H
    n = N // _CH
    c = (D**-0.5) * _LOG2E

    def kernel_function(q_hbm, k_hbm, v_hbm, o_hbm, qo_buf, k_buf, v_buf, rsem, wsem):
        def reads(i):
            slot = i % _W
            src = pl.ds(i * _CH, _CH)
            ring = pl.ds((i % _R) * _CH, _CH)
            return (
                pltpu.make_async_copy(q_hbm.at[src], qo_buf.at[src], rsem.at[0, slot]),
                pltpu.make_async_copy(k_hbm.at[src], k_buf.at[ring], rsem.at[1, slot]),
                pltpu.make_async_copy(v_hbm.at[src], v_buf.at[ring], rsem.at[2, slot]),
            )

        def start_writes(lo, hi):
            for h in range(lo, hi, _WCH):
                rows = pl.ds(h, min(_WCH, hi - h))
                pltpu.make_async_copy(qo_buf.at[rows], o_hbm.at[rows], wsem.at[0]).start()

        def compute(i):
            for h in range(_CH):
                hq = i * _CH + h
                hk = (i % _R) * _CH + h
                qo_buf[hq] = _head_attention(qo_buf[hq], k_buf[hk], v_buf[hk], c)

        for i in range(_W):
            for copy in reads(i):
                copy.start()

        def body(i, _):
            for copy in reads(i):
                copy.wait()

            @pl.when(i + _W < n)
            def _():
                for copy in reads(i + _W):
                    copy.start()

            compute(i)

        n0 = n - _E
        lax.fori_loop(0, n0, body, None)
        for i in range(n0, n):
            for copy in reads(i):
                copy.wait()
            if i == n0:
                start_writes(0, n0 * _CH)
            compute(i)
            start_writes(i * _CH, (i + 1) * _CH)
        pltpu.make_async_copy(qo_buf, o_hbm, wsem.at[0]).wait()

    out = pl.pallas_call(
        kernel_function,
        in_specs=[pl.BlockSpec(memory_space=pl.ANY)] * 3,
        out_specs=pl.BlockSpec(memory_space=pl.ANY),
        out_shape=jax.ShapeDtypeStruct((N, Sq, D), q.dtype),
        scratch_shapes=[
            pltpu.VMEM((N, Sq, D), q.dtype),
            pltpu.VMEM((_R * _CH, Sk, D), k.dtype),
            pltpu.VMEM((_R * _CH, Sk, D), v.dtype),
            pltpu.SemaphoreType.DMA((3, _W)),
            pltpu.SemaphoreType.DMA((1,)),
        ],
        compiler_params=pltpu.CompilerParams(vmem_limit_bytes=64 * 1024 * 1024),
    )(q.reshape(N, Sq, D), k.reshape(N, Sk, D), v.reshape(N, Sk, D))
    return out.reshape(B, H, Sq, D)
```

```python
import jax
import jax.numpy as jnp
from jax import lax
import jax.experimental.pallas as pl
import jax.experimental.pallas.tpu as pltpu

_LOG2E = 1.4426950408889634

_G = 4
_CR = 32
_W = 4
_R = 8
_E = 2
_WCR = 32
_WW = 16


def _head_attention(q, k, v, c):
    s = lax.dot_general(
        q, k, (((1,), (1,)), ((), ())), preferred_element_type=jnp.float32
    )
    m = jnp.max(s, axis=-1, keepdims=True)
    p = jnp.exp2((s - m) * c)
    l = jnp.sum(p, axis=-1, keepdims=True)
    o = jnp.dot(p.astype(v.dtype), v, preferred_element_type=jnp.float32)
    return (o * (1.0 / l)).astype(v.dtype)


@jax.jit
def pallas_standalone__mha_softmax__near_ridge_kernel(
    q: jax.Array,
    k: jax.Array,
    v: jax.Array,
):
    B, H, Sq, D = q.shape
    Sk = k.shape[2]
    groups = B // _G
    n = H * groups
    q_reads, kv_reads = Sq // _CR, Sk // _CR
    h_writes = Sq // _WCR
    n_writes = H * h_writes
    c = (D**-0.5) * _LOG2E

    def kernel_function(q_hbm, k_hbm, v_hbm, o_hbm, qo_buf, k_buf, v_buf, rsem, wsem):
        def unit(u):
            return u // groups, (u % groups) * _G

        def q_copy(u, rows):
            h, b0 = unit(u)
            idx = (pl.ds(b0, _G), h, rows)
            return pltpu.make_async_copy(q_hbm.at[idx], qo_buf.at[idx], rsem.at[0, u % _W])

        def kv_copies(u, rows):
            h, b0 = unit(u)
            idx = (pl.ds(b0, _G), h, rows)
            ring = (u % _R, slice(None), rows)
            return (
                pltpu.make_async_copy(k_hbm.at[idx], k_buf.at[ring], rsem.at[1, u % _W]),
                pltpu.make_async_copy(v_hbm.at[idx], v_buf.at[ring], rsem.at[2, u % _W]),
            )

        def start_reads(u):
            issued = 0
            for r in range(max(q_reads, kv_reads)):
                rows = pl.ds(r * _CR, _CR)
                copies = [q_copy(u, rows)] if r < q_reads else []
                if r < kv_reads:
                    copies += kv_copies(u, rows)
                for copy in copies:
                    copy.start(priority=issued % 2)
                    issued += 1

        def wait_reads(u):
            for copy in (q_copy(u, slice(None)), *kv_copies(u, slice(None))):
                copy.wait()

        def write(j):
            rows = pl.ds(pl.multiple_of((j % h_writes) * _WCR, _WCR), _WCR)
            idx = (slice(None), j // h_writes, rows)
            return pltpu.make_async_copy(qo_buf.at[idx], o_hbm.at[idx], wsem.at[j % _WW])

        for u in range(_W):
            start_reads(u)

        def read_and_compute(u, _):
            wait_reads(u)

            @pl.when(u + _W < n)
            def _():
                start_reads(u + _W)

            @pl.when(u == n - _E)
            def _():
                for j in range(_WW):
                    write(j).start()

            h, b0 = unit(u)
            for g in range(_G):
                qo_buf[b0 + g, h] = _head_attention(
                    qo_buf[b0 + g, h], k_buf[u % _R, g], v_buf[u % _R, g], c
                )

        lax.fori_loop(0, n, read_and_compute, None)

        def drain_writes(j, _):
            write(j).wait()

            @pl.when(j + _WW < n_writes)
            def _():
                write(j + _WW).start()

        lax.fori_loop(0, n_writes, drain_writes, None)

    return pl.pallas_call(
        kernel_function,
        in_specs=[pl.BlockSpec(memory_space=pl.ANY)] * 3,
        out_specs=pl.BlockSpec(memory_space=pl.ANY),
        out_shape=jax.ShapeDtypeStruct(q.shape, q.dtype),
        scratch_shapes=[
            pltpu.VMEM(q.shape, q.dtype),
            pltpu.VMEM((_R, _G, Sk, D), k.dtype),
            pltpu.VMEM((_R, _G, Sk, D), v.dtype),
            pltpu.SemaphoreType.DMA((3, _W)),
            pltpu.SemaphoreType.DMA((_WW,)),
        ],
        compiler_params=pltpu.CompilerParams(vmem_limit_bytes=64 * 1024 * 1024),
    )(q, k, v)
```

```python
import jax
import jax.numpy as jnp
from jax import lax
import jax.experimental.pallas as pl
import jax.experimental.pallas.tpu as pltpu

_LOG2E = 1.4426950408889634

_G = 2
_P = 2
_U = _G * _P
_CR = 32
_SHIFT = 3
_W = 3
_R = _W + 2
_E = 2
_WCR = 32
_WW = 16


def _head_attention(q, k, v, c):
    s = lax.dot_general(
        q, k, (((1,), (1,)), ((), ())), preferred_element_type=jnp.float32
    )
    m = jnp.max(s, axis=-1, keepdims=True)
    p = jnp.exp2((s - m) * c)
    l = jnp.sum(p, axis=-1, keepdims=True)
    o = jnp.dot(p.astype(v.dtype), v, preferred_element_type=jnp.float32)
    r = pltpu.reciprocal(l, approx=False, full_range=False)
    return (o * r).astype(v.dtype)


@jax.jit
def pallas_standalone__mha_softmax__near_ridge_kernel(
    q: jax.Array,
    k: jax.Array,
    v: jax.Array,
):
    B, H, S, D = q.shape
    groups = B // _U
    n = H * groups
    n_r = S // _CR
    h_writes = S // _WCR
    n_writes = H * h_writes
    c = (D**-0.5) * _LOG2E

    def kernel_function(q_hbm, k_hbm, v_hbm, o_hbm, qo_buf, k_buf, v_buf, rsem, wsem):
        hbm = (q_hbm, k_hbm, v_hbm)

        def read(u, j, p=None, r=None):
            h, b0 = u // groups, (u % groups) * _U
            rows = slice(None) if r is None else pl.ds(r * _CR, _CR)
            if p is None:
                bs, gs = pl.ds(b0, _U), slice(None)
            else:
                bs, gs = pl.ds(b0 + p * _G, _G), pl.ds(p * _G, _G)
            if j == 0:
                dst = qo_buf.at[bs, h, rows]
            else:
                dst = (k_buf, v_buf)[j - 1].at[u % _R, gs, rows]
            return pltpu.make_async_copy(hbm[j].at[bs, h, rows], dst, rsem.at[j, u % _W])

        def start_reads(u):
            for p in range(_P):
                for r in range(n_r):
                    for j, queue in enumerate((0, r % 2, 1)):
                        read(u, j, p, (r + j * _SHIFT) % n_r).start(priority=queue)

        def write(i):
            rows = pl.ds(pl.multiple_of((i % h_writes) * _WCR, _WCR), _WCR)
            idx = (slice(None), i // h_writes, rows)
            return pltpu.make_async_copy(qo_buf.at[idx], o_hbm.at[idx], wsem.at[i % _WW])

        for u in range(_W):
            start_reads(u)

        def read_and_compute(u, _):
            for j in range(3):
                read(u, j).wait()

            @pl.when(u + _W < n)
            def _():
                start_reads(u + _W)

            @pl.when(u == n - _E)
            def _():
                for i in range(_WW):
                    write(i).start()

            h, b0 = u // groups, (u % groups) * _U
            for g in range(_U):
                qo_buf[b0 + g, h] = _head_attention(
                    qo_buf[b0 + g, h], k_buf[u % _R, g], v_buf[u % _R, g], c
                )

        lax.fori_loop(0, n, read_and_compute, None)

        def drain_writes(i, _):
            write(i).wait()

            @pl.when(i + _WW < n_writes)
            def _():
                write(i + _WW).start()

        lax.fori_loop(0, n_writes, drain_writes, None)

    return pl.pallas_call(
        kernel_function,
        in_specs=[pl.BlockSpec(memory_space=pl.ANY)] * 3,
        out_specs=pl.BlockSpec(memory_space=pl.ANY),
        out_shape=jax.ShapeDtypeStruct(q.shape, q.dtype),
        scratch_shapes=[
            pltpu.VMEM(q.shape, q.dtype),
            pltpu.VMEM((_R, _U, S, D), k.dtype),
            pltpu.VMEM((_R, _U, S, D), v.dtype),
            pltpu.SemaphoreType.DMA((3, _W)),
            pltpu.SemaphoreType.DMA((_WW,)),
        ],
        compiler_params=pltpu.CompilerParams(
            vmem_limit_bytes=64 * 1024 * 1024,
            disable_bounds_checks=True,
        ),
    )(q, k, v)
```

```python
import jax
import jax.numpy as jnp
from jax import lax
import jax.experimental.pallas as pl
import jax.experimental.pallas.tpu as pltpu

_LOG2E = 1.4426950408889634

_G = 2
_P = 2
_U = _G * _P
_CR = 32
_QUEUES = (0, 1, 0, 1, 1)
_W = 3
_R = _W + 1
_E = 3
_WCR = 32
_WW = 6
_TOPUP = 5


def _head_attention(q, k, v, c):
    s = lax.dot_general(
        q, k, (((1,), (1,)), ((), ())), preferred_element_type=jnp.float32
    )
    m = jnp.max(s, axis=-1, keepdims=True)
    p = jnp.exp2((s - m) * c)
    l = jnp.sum(p, axis=-1, keepdims=True)
    o = jnp.dot(p.astype(v.dtype), v, preferred_element_type=jnp.float32)
    r = pltpu.reciprocal(l, approx=False, full_range=False)
    return (o * r).astype(v.dtype)


@jax.jit
def pallas_standalone__mha_softmax__near_ridge_kernel(
    q: jax.Array,
    k: jax.Array,
    v: jax.Array,
):
    B, H, S, D = q.shape
    groups = B // _U
    n = H * groups
    n_r = S // _CR
    h_writes = S // _WCR
    n_writes = H * h_writes
    first_write_unit = n - _E
    c = (D**-0.5) * _LOG2E

    def kernel_function(q_hbm, k_hbm, v_hbm, o_hbm, qo_buf, k_buf, v_buf, rsem, wsem):
        hbm = (q_hbm, k_hbm, v_hbm)

        def read(u, j, p=None, r=None):
            h, b0 = u // groups, (u % groups) * _U
            rows = slice(None) if r is None else pl.ds(r * _CR, _CR)
            if p is None:
                bs, gs = pl.ds(b0, _U), slice(None)
            else:
                bs, gs = pl.ds(b0 + p * _G, _G), pl.ds(p * _G, _G)
            if j == 0:
                dst = qo_buf.at[bs, h, rows]
            else:
                dst = (k_buf, v_buf)[j - 1].at[u % _R, gs, rows]
            return pltpu.make_async_copy(hbm[j].at[bs, h, rows], dst, rsem.at[j, u % _W])

        def start_reads(u):
            for p in range(_P):
                for r in range(n_r):
                    for j in range(3):
                        queue = _QUEUES[(3 * r + j) % len(_QUEUES)]
                        read(u, j, p, r).start(priority=queue)

        def write(i):
            rows = pl.ds(pl.multiple_of((i % h_writes) * _WCR, _WCR), _WCR)
            idx = (slice(None), i // h_writes, rows)
            return pltpu.make_async_copy(qo_buf.at[idx], o_hbm.at[idx], wsem.at[i % _WW])

        def start_writes():
            for i in range(_WW):
                write(i).start()

        for u in range(_W):
            start_reads(u)

        def read_and_compute(u, _):
            for j in range(3):
                read(u, j).wait()

            @pl.when(u + _W < n)
            def _():
                start_reads(u + _W)

            @pl.when(u > first_write_unit)
            def _():
                for t in range(_TOPUP):
                    i = (u - first_write_unit - 1) * _TOPUP + t
                    write(i).wait()
                    write(i + _WW).start()

            h, b0 = u // groups, (u % groups) * _U
            for g in range(_U):
                if g == _U - 1:
                    pl.when(u == first_write_unit)(start_writes)
                qo_buf[b0 + g, h] = _head_attention(
                    qo_buf[b0 + g, h], k_buf[u % _R, g], v_buf[u % _R, g], c
                )

        lax.fori_loop(0, n, read_and_compute, None)

        def drain_writes(i, _):
            write(i).wait()

            @pl.when(i + _WW < n_writes)
            def _():
                write(i + _WW).start()

        lax.fori_loop((_E - 1) * _TOPUP, n_writes, drain_writes, None)

    return pl.pallas_call(
        kernel_function,
        in_specs=[pl.BlockSpec(memory_space=pl.ANY)] * 3,
        out_specs=pl.BlockSpec(memory_space=pl.ANY),
        out_shape=jax.ShapeDtypeStruct(q.shape, q.dtype),
        scratch_shapes=[
            pltpu.VMEM(q.shape, q.dtype),
            pltpu.VMEM((_R, _U, S, D), k.dtype),
            pltpu.VMEM((_R, _U, S, D), v.dtype),
            pltpu.SemaphoreType.DMA((3, _W)),
            pltpu.SemaphoreType.DMA((_WW,)),
        ],
        compiler_params=pltpu.CompilerParams(
            vmem_limit_bytes=64 * 1024 * 1024,
            disable_bounds_checks=True,
        ),
    )(q, k, v)
```

```python
import jax
import jax.numpy as jnp
from jax import lax
import jax.experimental.pallas as pl
import jax.experimental.pallas.tpu as pltpu

_LOG2E = 1.4426950408889634

_G = 2
_P = 2
_U = _G * _P
_CR = 32
_QUEUES = (0, 1, 0, 1, 1)
_W = 3
_R = _W + 1
_WCR = 32
_WH = 2
_E = 3


def _head_attention(q, k, v, c):
    s = lax.dot_general(
        q, k, (((1,), (1,)), ((), ())), preferred_element_type=jnp.float32
    )
    m = jnp.max(s, axis=-1, keepdims=True)
    p = jnp.exp2((s - m) * c)
    l = jnp.sum(p, axis=-1, keepdims=True)
    o = jnp.dot(p.astype(v.dtype), v, preferred_element_type=jnp.float32)
    r = pltpu.reciprocal(l, approx=False, full_range=False)
    return (o * r).astype(v.dtype)


@jax.jit
def pallas_standalone__mha_softmax__near_ridge_kernel(
    q: jax.Array,
    k: jax.Array,
    v: jax.Array,
):
    B, H, Sq, D = q.shape
    Sk = k.shape[2]
    groups = B // _U
    n = H * groups
    first_write_unit = n - _E
    c = (D**-0.5) * _LOG2E
    assert B % _U == 0 and Sq % _CR == 0 and Sk % _CR == 0 and Sq % _WCR == 0
    assert n >= max(_W, _E)
    assert _WH + _E - 1 <= first_write_unit // groups

    def kernel_function(q_hbm, k_hbm, v_hbm, o_hbm, qo_buf, k_buf, v_buf, rsem, wsem):
        hbm = (q_hbm, k_hbm, v_hbm)
        n_slices = (Sq // _CR, Sk // _CR, Sk // _CR)

        def read(u, j, p=None, r=None):
            h, b0 = u // groups, (u % groups) * _U
            rows = slice(None) if r is None else pl.ds(r * _CR, _CR)
            if p is None:
                bs, gs = pl.ds(b0, _U), slice(None)
            else:
                bs, gs = pl.ds(b0 + p * _G, _G), pl.ds(p * _G, _G)
            if j == 0:
                dst = qo_buf.at[bs, h, rows]
            else:
                dst = (k_buf, v_buf)[j - 1].at[u % _R, gs, rows]
            return pltpu.make_async_copy(hbm[j].at[bs, h, rows], dst, rsem.at[j, u % _W])

        def start_reads(u):
            for p in range(_P):
                for r in range(max(n_slices)):
                    for j in range(3):
                        if r < n_slices[j]:
                            queue = _QUEUES[(3 * r + j) % len(_QUEUES)]
                            read(u, j, p, r).start(priority=queue)

        def write(h, r=None):
            rows = slice(None) if r is None else pl.ds(r * _WCR, _WCR)
            idx = (slice(None), h, rows)
            return pltpu.make_async_copy(qo_buf.at[idx], o_hbm.at[idx], wsem.at[h % _WH])

        def start_writes(h):
            for r in range(Sq // _WCR):
                write(h, r).start()

        def advance_writes(h):
            write(h).wait()

            @pl.when(h + _WH < H)
            def _():
                start_writes(h + _WH)

        for u in range(_W):
            start_reads(u)

        def read_and_compute(u, _):
            for j in range(3):
                read(u, j).wait()

            @pl.when(u + _W < n)
            def _():
                start_reads(u + _W)

            @pl.when(u > first_write_unit)
            def _():
                advance_writes(u - first_write_unit - 1)

            h, b0 = u // groups, (u % groups) * _U
            for g in range(_U):
                if g == _U - 1:

                    @pl.when(u == first_write_unit)
                    def _():
                        for h_out in range(_WH):
                            start_writes(h_out)

                qo_buf[b0 + g, h] = _head_attention(
                    qo_buf[b0 + g, h], k_buf[u % _R, g], v_buf[u % _R, g], c
                )

        lax.fori_loop(0, n, read_and_compute, None)
        lax.fori_loop(_E - 1, H, lambda h, _: advance_writes(h), None)

    return pl.pallas_call(
        kernel_function,
        in_specs=[pl.BlockSpec(memory_space=pl.ANY)] * 3,
        out_specs=pl.BlockSpec(memory_space=pl.ANY),
        out_shape=jax.ShapeDtypeStruct(q.shape, q.dtype),
        scratch_shapes=[
            pltpu.VMEM(q.shape, q.dtype),
            pltpu.VMEM((_R, _U, Sk, D), k.dtype),
            pltpu.VMEM((_R, _U, Sk, D), v.dtype),
            pltpu.SemaphoreType.DMA((3, _W)),
            pltpu.SemaphoreType.DMA((_WH,)),
        ],
        compiler_params=pltpu.CompilerParams(
            vmem_limit_bytes=64 * 1024 * 1024,
            disable_bounds_checks=True,
        ),
    )(q, k, v)
```

```python
import jax
import jax.numpy as jnp
from jax import lax
import jax.experimental.pallas as pl
import jax.experimental.pallas.tpu as pltpu

_LOG2E = 1.4426950408889634

_U = 4
_CR = 64
_W = 3
_R = _W + 1
_WCR = 32
_WH = 2
_E = 3
_EPOS = 3


def _head_attention(q, k, v, c):
    s = lax.dot_general(
        q, k, (((1,), (1,)), ((), ())), preferred_element_type=jnp.float32
    )
    m = jnp.max(s, axis=-1, keepdims=True)
    p = jnp.exp2((s - m) * c)
    l = jnp.sum(p, axis=-1, keepdims=True)
    o = jnp.dot(p.astype(v.dtype), v, preferred_element_type=jnp.float32)
    return (o * (1.0 / l)).astype(v.dtype)


@jax.jit
def pallas_standalone__mha_softmax__near_ridge_kernel(
    q: jax.Array,
    k: jax.Array,
    v: jax.Array,
):
    B, H, Sq, D = q.shape
    Sk = k.shape[2]
    C = B // _U
    n = H * C
    first_write_unit = n - _E
    c = (D**-0.5) * _LOG2E
    assert B % _U == 0 and Sq % _CR == 0 and Sk % _CR == 0 and Sq % _WCR == 0
    assert n >= max(_W, _E)
    assert _WH + _E - 1 <= first_write_unit // C

    def kernel_function(q_hbm, k_hbm, v_hbm, o_hbm, qo_buf, k_buf, v_buf, rsem, wsem):
        hbm = (q_hbm, k_hbm, v_hbm)
        n_slices = (Sq // _CR, Sk // _CR, Sk // _CR)

        def unit_bufs(u):
            return qo_buf.at[u // C, :, u % C], k_buf.at[u % _R], v_buf.at[u % _R]

        def start_reads(u):
            h, i = u // C, u % C
            bufs = unit_bufs(u)
            issued = 0
            for r in range(max(n_slices)):
                rows = pl.ds(r * _CR, _CR)
                for j in (2, 1, 0):
                    if r >= n_slices[j]:
                        continue
                    for p in range(_U):
                        pltpu.make_async_copy(
                            hbm[j].at[p * C + i, h, rows],
                            bufs[j].at[p, rows],
                            rsem.at[j, u % _W],
                        ).start(priority=issued % 2)
                        issued += 1

        def wait_reads(u):
            for j, buf in enumerate(unit_bufs(u)):
                pltpu.make_async_copy(buf, buf, rsem.at[j, u % _W]).wait()

        def start_writes(h):
            for r in range(Sq // _WCR):
                rows = pl.ds(r * _WCR, _WCR)
                for p in range(_U):
                    pltpu.make_async_copy(
                        qo_buf.at[h, p, :, rows],
                        o_hbm.at[pl.ds(p * C, C), h, rows],
                        wsem.at[h % _WH],
                    ).start()

        def advance_writes(h):
            pltpu.make_async_copy(qo_buf.at[h], qo_buf.at[h], wsem.at[h % _WH]).wait()

            @pl.when(h + _WH < H)
            def _():
                start_writes(h + _WH)

        for u in range(_W):
            start_reads(u)

        def read_and_compute(u, _):
            wait_reads(u)

            @pl.when(u + _W < n)
            def _():
                start_reads(u + _W)

            @pl.when(u > first_write_unit)
            def _():
                advance_writes(u - first_write_unit - 1)

            for p in range(_U):
                if p == _EPOS:

                    @pl.when(u == first_write_unit)
                    def _():
                        for h_out in range(_WH):
                            start_writes(h_out)

                tile = (u // C, p, u % C)
                qo_buf[tile] = _head_attention(
                    qo_buf[tile], k_buf[u % _R, p], v_buf[u % _R, p], c
                )

        lax.fori_loop(0, n, read_and_compute, None)
        lax.fori_loop(_E - 1, H, lambda h, _: advance_writes(h), None)

    return pl.pallas_call(
        kernel_function,
        in_specs=[pl.BlockSpec(memory_space=pl.ANY)] * 3,
        out_specs=pl.BlockSpec(memory_space=pl.ANY),
        out_shape=jax.ShapeDtypeStruct(q.shape, q.dtype),
        scratch_shapes=[
            pltpu.VMEM((H, _U, C, Sq, D), q.dtype),
            pltpu.VMEM((_R, _U, Sk, D), k.dtype),
            pltpu.VMEM((_R, _U, Sk, D), v.dtype),
            pltpu.SemaphoreType.DMA((3, _W)),
            pltpu.SemaphoreType.DMA((_WH,)),
        ],
        compiler_params=pltpu.CompilerParams(
            vmem_limit_bytes=64 * 1024 * 1024,
            disable_bounds_checks=True,
        ),
    )(q, k, v)
```
